```python
import os as _os
_os.environ.setdefault("JAX_PLATFORMS", "cpu")
import jax
import jax.numpy as jnp

def _softmax(x, axis=-1):
    return jax.nn.softmax(x, axis=axis)
def _gelu(x):
    return jax.nn.gelu(x, approximate=True)
def _silu(x):
    return jax.nn.silu(x)
def _sigmoid(x):
    return jax.nn.sigmoid(x)
def _layernorm(x, axis=-1, eps=1e-5):
    m = jnp.mean(x, axis=axis, keepdims=True)
    v = jnp.var(x, axis=axis, keepdims=True)
    return (x - m) / jnp.sqrt(v + eps)
def _scatter_add(tgt, idx, src, axis=0):
    return tgt.at[idx].add(src)
def _segment_sum(src, seg, n):
    return jax.ops.segment_sum(src, seg, n)
class _Rng:
    def __init__(self, key):
        self._k = key
    def _next(self):
        self._k, sub = jax.random.split(self._k)
        return sub
    def normal(self, shape):
        return jax.random.normal(self._next(), shape, dtype=jnp.bfloat16)
    def randint(self, lo, hi, shape):
        return jax.random.randint(self._next(), shape, lo, hi, dtype=jnp.int32)
    def uniform(self, shape, lo=0.0, hi=1.0):
        return jax.random.uniform(self._next(), shape, jnp.bfloat16, lo, hi)
    def permutation(self, n):
        return jax.random.permutation(self._next(), n)


kernel_name = 'concat_heads__sliding_block_cached__sliding_block_cached__decode'

def setup_inputs():
    _rng = _Rng(jax.random.key(int.from_bytes(__import__("os").urandom(4), "little")))
    _w = (lambda a: (lambda t: t.astype(jnp.bfloat16) if jnp.issubdtype(t.dtype, jnp.floating) else t)(jnp.asarray(a)))
    def _A_setup():
        B, Sq, D = 4, 1, 576
        Hq, Hkv, Sk, Dh = 32, 16, 8192, 128
        assert Hq % Hkv == 0, (Hq, Hkv)
        return {
            "x": _w((lambda *s: _rng.normal(s) * 0.8)(B, Sq, D)),
            "k_cache": _w((lambda *s: _rng.normal(s) * 0.8)(B, Hkv, Sk, Dh)),
            "v_cache": _w((lambda *s: _rng.normal(s) * 0.05)(B, Hkv, Sk, Dh)),
            "wq": _w((lambda *s: _rng.normal(s) * 0.8)(D, Hq * Dh) * (D ** -0.5)),
            "wo": _w((lambda *s: _rng.normal(s) * 0.05)(Hq * Dh, D) * ((Hq * Dh) ** -0.5)),
        }
    _A_in = _A_setup()

    def _B_setup():
        B, Sq, D = 4, 1, 576
        Hq, Hkv, Sk, Dh = 32, 16, 8192, 128
        assert Hq % Hkv == 0, (Hq, Hkv)
        return {
            "x": _w((lambda *s: _rng.normal(s) * 0.8)(B, Sq, D)),
            "k_cache": _w((lambda *s: _rng.normal(s) * 0.8)(B, Hkv, Sk, Dh)),
            "v_cache": _w((lambda *s: _rng.normal(s) * 0.05)(B, Hkv, Sk, Dh)),
            "wq": _w((lambda *s: _rng.normal(s) * 0.8)(D, Hq * Dh) * (D ** -0.5)),
            "wo": _w((lambda *s: _rng.normal(s) * 0.05)(Hq * Dh, D) * ((Hq * Dh) ** -0.5)),
        }
    _B_in = _B_setup()

    return {
        "A_x": _A_in["x"],
        "A_k_cache": _A_in["k_cache"],
        "A_v_cache": _A_in["v_cache"],
        "A_wq": _A_in["wq"],
        "A_wo": _A_in["wo"],
        "B_x": _B_in["x"],
        "B_k_cache": _B_in["k_cache"],
        "B_v_cache": _B_in["v_cache"],
        "B_wq": _B_in["wq"],
        "B_wo": _B_in["wo"],
    }

def reference(A_x, A_k_cache, A_v_cache, A_wq, A_wo, B_x, B_k_cache, B_v_cache, B_wq, B_wo):
    def _A_ref(x, k_cache, v_cache, wq, wo):
        B, Sq, D = x.shape
        Hq, Dh = 32, 128
        Hkv, Sk = k_cache.shape[1], k_cache.shape[2]
        W = min(4096, max(256, Sk // 4))
        rep = Hq // Hkv
        q = (lambda x, *d: x.transpose(*d))((x @ wq).reshape(B, Sq, Hq, Dh), 0, 2, 1, 3)
        k = jnp.repeat(k_cache[:, :, Sk - W:, :], rep, axis=1)
        v = jnp.repeat(v_cache[:, :, Sk - W:, :], rep, axis=1)
        scores = jnp.einsum("bhqd,bhkd->bhqk", q, k) * (Dh ** -0.5)
        p = _softmax(scores, axis=-1)
        o = jnp.einsum("bhqk,bhkd->bhqd", p, v)
        return (lambda x, *d: x.transpose(*d))(o, 0, 2, 1, 3).reshape(B, Sq, Hq * Dh) @ wo

    def _B_ref(x, k_cache, v_cache, wq, wo):
        B, Sq, D = x.shape
        Hq, Dh = 32, 128
        Hkv, Sk = k_cache.shape[1], k_cache.shape[2]
        W = min(4096, max(256, Sk // 4))
        rep = Hq // Hkv
        q = (lambda x, *d: x.transpose(*d))((x @ wq).reshape(B, Sq, Hq, Dh), 0, 2, 1, 3)
        k = jnp.repeat(k_cache[:, :, Sk - W:, :], rep, axis=1)
        v = jnp.repeat(v_cache[:, :, Sk - W:, :], rep, axis=1)
        scores = jnp.einsum("bhqd,bhkd->bhqk", q, k) * (Dh ** -0.5)
        p = _softmax(scores, axis=-1)
        o = jnp.einsum("bhqk,bhkd->bhqd", p, v)
        return (lambda x, *d: x.transpose(*d))(o, 0, 2, 1, 3).reshape(B, Sq, Hq * Dh) @ wo

    a = _A_ref(A_x, A_k_cache, A_v_cache, A_wq, A_wo)
    b = _B_ref(B_x, B_k_cache, B_v_cache, B_wq, B_wo)
    return jnp.concatenate([a, b], axis=-1)
```

```python
import functools
import jax
import jax.numpy as jnp
from jax import lax
import jax.experimental.pallas as pl
import jax.experimental.pallas.tpu as pltpu

_HQ = 32
_DH = 128
_NT = (((1,), (1,)), ((), ()))


def _kernel(xa, ka, va, wqa, woa, xb, kb, vb, wqb, wob, out_ref,
            x_buf, wq_buf, wo_buf, k_buf, v_buf, q_buf, o_buf,
            x_sem, wq_sem, wo_sem, k_sem, v_sem, *, nb, hkv, sk, w, nbuf):
    xs, ks, vs, wqs, wos = (xa, xb), (ka, kb), (va, vb), (wqa, wqb), (woa, wob)
    d = xa.shape[-1]
    rows = 2 * nb

    def x_copy(br):
        return pltpu.make_async_copy(xs[br], x_buf.at[br], x_sem.at[br])

    def wq_copy(br):
        return pltpu.make_async_copy(wqs[br], wq_buf.at[br], wq_sem.at[br])

    def wo_copy(br):
        return pltpu.make_async_copy(wos[br], wo_buf.at[br], wo_sem.at[br])

    def kv_copy(src, buf, sem, h, slot):
        return pltpu.make_async_copy(
            src.at[:, h, pl.ds(sk - w, w), :], buf.at[slot], sem.at[slot])

    def start_kv(br, h, slot):
        kv_copy(ks[br], k_buf, k_sem, h, slot).start(priority=0)
        kv_copy(vs[br], v_buf, v_sem, h, slot).start(priority=1)

    x_copy(0).start()
    x_copy(1).start()
    wq_copy(0).start()
    for i in range(nbuf):
        start_kv(0, i, i)
    wq_copy(1).start()
    wo_copy(0).start(priority=1)

    row_id = lax.broadcasted_iota(jnp.int32, (rows, _DH), 0)

    def q_proj(br):
        x_copy(br).wait()
        wq_copy(br).wait()
        x = x_buf[br].astype(jnp.float32)
        x2 = jnp.concatenate([x, x], axis=0).astype(jnp.bfloat16)
        for h in range(hkv):
            q2 = jnp.dot(x2, wq_buf[br, :, 2 * h * _DH:(2 * h + 2) * _DH],
                         preferred_element_type=jnp.float32)
            q_buf[br, h] = jnp.where(row_id < nb, q2[:, :_DH], q2[:, _DH:])

    def attend(br, h):
        g = br * hkv + h
        slot = g % nbuf
        q = q_buf[br, h].astype(jnp.bfloat16)
        kv_copy(ks[br], k_buf, k_sem, h, slot).wait()
        row_s = lax.broadcasted_iota(jnp.int32, (rows, w), 0) % nb
        s = None
        for b in range(nb):
            sb = lax.dot_general(q, k_buf[slot, b], _NT,
                                 preferred_element_type=jnp.float32)
            s = sb if s is None else jnp.where(row_s == b, sb, s)
        s = s * (_DH ** -0.5)
        m = jnp.max(s, axis=-1, keepdims=True)
        e = jnp.exp(s - m)
        l = jnp.sum(e, axis=-1, keepdims=True)
        p = e.astype(jnp.bfloat16)
        kv_copy(vs[br], v_buf, v_sem, h, slot).wait()
        o = None
        for b in range(nb):
            ob = jnp.dot(p, v_buf[slot, b], preferred_element_type=jnp.float32)
            o = ob if o is None else jnp.where(row_id % nb == b, ob, o)
        o_buf[br, h] = o / l
        nxt = g + nbuf
        if br == 0:
            @pl.when(nxt < hkv)
            def _():
                start_kv(0, nxt, slot)

            @pl.when(nxt >= hkv)
            def _():
                start_kv(1, nxt - hkv, slot)
        else:
            @pl.when(nxt < 2 * hkv)
            def _():
                start_kv(1, nxt - hkv, slot)

            @pl.when(nxt == 2 * hkv)
            def _():
                wo_copy(1).start()

    def o_proj(br):
        parts = []
        for h in range(hkv):
            o = o_buf[br, h]
            parts.append(o)
            parts.append(pltpu.roll(o, nb, 0))
        o_all = jnp.concatenate(parts, axis=1).astype(jnp.bfloat16)
        wo_copy(br).wait()
        y = lax.dot_general(o_all, wo_buf[br], _NT,
                            preferred_element_type=jnp.float32)
        return y[:nb]

    q_proj(0)
    lax.fori_loop(0, hkv, lambda h, c: attend(0, h), None)
    q_proj(1)
    ya = o_proj(0)
    lax.fori_loop(0, hkv, lambda h, c: attend(1, h), None)
    yb = o_proj(1)
    out_ref[...] = jnp.concatenate([ya, yb], axis=1).astype(out_ref.dtype)


@jax.jit
def pallas_concat_heads__sliding_block_cached__sliding_block_cached__decode_kernel(
    A_x: jax.Array,
    A_k_cache: jax.Array,
    A_v_cache: jax.Array,
    A_wq: jax.Array,
    A_wo: jax.Array,
    B_x: jax.Array,
    B_k_cache: jax.Array,
    B_v_cache: jax.Array,
    B_wq: jax.Array,
    B_wo: jax.Array,
):
    nbuf = 4
    nb, sq, d = A_x.shape
    _, hkv, sk, dh = A_k_cache.shape
    w = min(4096, max(256, sk // 4))
    bf = jnp.bfloat16
    hbm = pl.BlockSpec(memory_space=pltpu.HBM)
    out = pl.pallas_call(
        functools.partial(_kernel, nb=nb, hkv=hkv, sk=sk, w=w, nbuf=nbuf),
        out_shape=jax.ShapeDtypeStruct((nb, 2 * d), bf),
        in_specs=[hbm] * 10,
        out_specs=pl.BlockSpec(memory_space=pltpu.VMEM),
        scratch_shapes=[
            pltpu.VMEM((2, nb, d), bf),
            pltpu.VMEM((2, d, _HQ * _DH), bf),
            pltpu.VMEM((2, d, _HQ * _DH), bf),
            pltpu.VMEM((nbuf, nb, w, _DH), bf),
            pltpu.VMEM((nbuf, nb, w, _DH), bf),
            pltpu.VMEM((2, hkv, 2 * nb, _DH), jnp.float32),
            pltpu.VMEM((2, hkv, 2 * nb, _DH), jnp.float32),
            pltpu.SemaphoreType.DMA((2,)),
            pltpu.SemaphoreType.DMA((2,)),
            pltpu.SemaphoreType.DMA((2,)),
            pltpu.SemaphoreType.DMA((nbuf,)),
            pltpu.SemaphoreType.DMA((nbuf,)),
        ],
        compiler_params=pltpu.CompilerParams(vmem_limit_bytes=100 * 1024 * 1024),
    )(A_x.reshape(nb, d), A_k_cache, A_v_cache, A_wq, A_wo.T,
      B_x.reshape(nb, d), B_k_cache, B_v_cache, B_wq, B_wo.T)
    return out.reshape(nb, sq, 2 * d)
```

```python
import functools

import jax
import jax.numpy as jnp
from jax import lax
import jax.experimental.pallas as pl
import jax.experimental.pallas.tpu as pltpu

_HQ = 32
_DH = 128
_G = 4
_BLK = 128
_KR = 64
_WR = 8
_WC = 1024
_BAND = 16
_QC = 256
_LOOK = 16
_NSLOT = 4
_NT = (((1,), (1,)), ((), ()))
_PIECES = ((0, 0, _G - 1, 1), (1, 1, _G - 1, 1), (0, _G - 1, 1, 0), (1, 0, 1, 0))


def _divmod(j, n):
    assert n & (n - 1) == 0
    return lax.shift_right_logical(j, n.bit_length() - 1), j & (n - 1)


def _ds(i, n):
    return pl.ds(i * n if isinstance(i, int) else pl.multiple_of(i * n, n), n)


def _stream(xa, ka, va, wqa, woa, xb, kb, vb, wqb, wob,
            x_buf, x8_buf, wq_buf, wo_buf, kv_buf, q_buf, s_buf, o_buf, lhs_buf,
            st_buf, y_buf, x_sem, sems):
    f32, bf16 = jnp.float32, jnp.bfloat16
    nb, d = xa.shape
    sk, w = ka.shape[1], kv_buf.shape[3]
    rows = 2 * nb
    ngrp = ka.shape[0] // _G
    nblk = w // _BLK
    nkv = ngrp * nblk
    ncol = _HQ * _DH // _WC
    nband = d // _G // _BAND
    nw = nband * ncol

    def w_unit(ref, r, c):
        return ref.at[(slice(None),) * (len(ref.shape) - 2) + (_ds(r, _WR), _ds(c, _WC))]

    def wq_unit(ref, n, s):
        return w_unit(ref, *_divmod(2 * n + s, ncol))

    def wo_unit(ref, n, s):
        r, c = _divmod(n, ncol)
        return w_unit(ref, 2 * r + s, c)

    def kv_dst(n, s):
        g, i = _divmod(n, nblk)
        return kv_buf.at[_divmod(g, _NSLOT)[1], :, :, _ds(2 * i + s, _KR), :]

    def kv_src(ref, n, s):
        g, i = _divmod(n, nblk)
        return ref.at[_ds(g, _G), _ds((sk - w) // _KR + 2 * i + s, _KR), :]

    def start(srcs, dst, sem):
        for a, l0, nl, queue in _PIECES:
            pltpu.make_async_copy(srcs[a].at[pl.ds(l0, nl)], dst.at[a, pl.ds(l0, nl)],
                                  sem).start(priority=queue)

    def wait(dst, sem):
        pltpu.make_async_copy(dst, dst, sem).wait()

    def sem_of(n, s):
        return sems.at[2 * _divmod(n, _LOOK)[1] + s]

    def start_wq(n, s, sem):
        start((wq_unit(wqa, n, s), wq_unit(wqb, n, s)), wq_unit(wq_buf, n, s), sem)

    def start_a(n, s, sem):
        start((kv_src(ka, n, s), kv_src(va, n, s)), kv_dst(n, s), sem)

    def start_b(n, s, sem):
        start((kv_src(kb, n - nkv, s), kv_src(vb, n - nkv, s)), kv_dst(n, s), sem)

    def start_wo(n, s, sem):
        start((wo_unit(woa, n, s), wo_unit(wob, n, s)), wo_unit(wo_buf, n, s), sem)

    x_copies = [pltpu.make_async_copy(x, x_buf.at[i], x_sem.at[i])
                for i, x in enumerate((xa, xb))]

    @pl.loop(0, _LOOK)
    def _(n):
        for s in range(2):
            start_wq(n, s, sem_of(n, s))

    for cp in x_copies:
        cp.start()

    @pl.loop(0, nw - _LOOK)
    def _(n):
        for s in range(2):
            wait(wq_unit(wq_buf, n, s), sem_of(n, s))
            start_wq(n + _LOOK, s, sem_of(n, s))

    @pl.loop(nw - _LOOK, nw)
    def _(n):
        for s in range(2):
            wait(wq_unit(wq_buf, n, s), sem_of(n, s))
            start_a(n - (nw - _LOOK), s, sem_of(n, s))

    for cp in x_copies:
        cp.wait()
    x8_buf[...] = jnp.concatenate([x_buf[0].astype(f32), x_buf[1].astype(f32)], axis=0)

    def q_step(n):
        x8 = x8_buf[...].astype(bf16)
        qa, qb = [jnp.dot(x8, wq_buf[br, :, :, _ds(n, _QC)].reshape(d, _QC),
                          preferred_element_type=f32) for br in range(2)]
        q = jnp.where(lax.broadcasted_iota(jnp.int32, qa.shape, 0) < nb, qa, qb)
        for h in range(_QC // _DH):
            q_buf[pl.ds(n * (_QC // _DH) + h, rows, stride=_HQ), :] = q[:, h * _DH:(h + 1) * _DH]

    nq = _HQ * _DH // _QC
    nq0 = rows * _DH // _QC
    assert nq - nq0 <= nblk
    pl.loop(0, nq0)(q_step)

    zeros = jnp.zeros((rows, _DH), f32)
    neg_inf = jnp.full((rows, _DH), -jnp.inf, f32)
    lane_of_row = lax.shift_right_logical(lax.broadcasted_iota(jnp.int32, (rows, _DH), 0), 1)
    M_PREV, M_RUN, L_ACC, O_ACC = range(4)
    st_buf[M_RUN] = neg_inf

    def pick(parts):
        out = parts[0]
        for l in range(1, _G):
            out = jnp.where(lane_of_row == l, parts[l], out)
        return out

    def pv_step(slot, i):
        e = jnp.exp(s_buf[i] - st_buf[M_PREV])
        p = e.astype(bf16)
        st_buf[L_ACC] += e
        st_buf[O_ACC] += pick([jnp.dot(p, kv_buf[slot, 1, l, _ds(i, _BLK), :],
                                       preferred_element_type=f32) for l in range(_G)])

    def finish(t):
        o_buf[_ds(t, rows), :] = st_buf[O_ACC] / jnp.sum(st_buf[L_ACC], axis=-1, keepdims=True)

    def attend(start_next, first, n):
        t, i = _divmod(n, nblk)

        def advance(s):
            sem = sem_of(n + nw, s)
            wait(kv_dst(n, s), sem)
            start_next(n + _LOOK, s, sem)

        advance(0)
        if first:
            pl.when(i + nq0 < nq)(lambda: q_step(i + nq0))
        else:
            pv_step(_divmod(t - 1, _NSLOT)[1], i)
        advance(1)
        q = q_buf[_ds(t, rows), :].astype(bf16)
        s = pick([lax.dot_general(q, kv_buf[_divmod(t, _NSLOT)[1], 0, l, _ds(i, _BLK), :], _NT,
                                  preferred_element_type=f32)
                  for l in range(_G)]) * (_DH ** -0.5)
        s_buf[i] = s
        st_buf[M_RUN] = jnp.maximum(st_buf[M_RUN], s)

        @pl.when(i == nblk - 1)
        def _():
            if not first:
                finish(t - 1)
            st_buf[M_PREV] = jnp.broadcast_to(
                jnp.max(st_buf[M_RUN], axis=-1, keepdims=True), (rows, _DH))
            st_buf[M_RUN] = neg_inf
            st_buf[L_ACC] = zeros
            st_buf[O_ACC] = zeros

    lo = 0
    for hi, start_next in ((nblk, start_a),
                           (nkv - _LOOK, start_a),
                           (2 * nkv - _LOOK, start_b),
                           (2 * nkv, lambda n, s, sem: start_wo(n - 2 * nkv, s, sem))):
        pl.loop(lo, hi)(functools.partial(attend, start_next, lo == 0))
        lo = hi

    last = 2 * ngrp - 1
    pl.loop(0, nblk, unroll=2)(functools.partial(pv_step, last % _NSLOT))
    finish(last)

    hpc = _WC // _DH
    for c in range(ncol):
        lhs_buf[c] = jnp.concatenate(
            [o_buf[pl.ds(c * hpc + h, rows, stride=_HQ), :] for h in range(hpc)], axis=1)

    ntile = 2 * d // _DH
    lane = lax.broadcasted_iota(jnp.int32, (rows, _DH), 1)
    seg = _divmod(lane, _BAND)[0]
    segs = [seg + (v * _DH // _BAND) % nband for v in range(ntile)]
    band_of_col = [jnp.where(x >= nband, x - nband, x) for x in segs]

    def band(j, ys):
        def step(c, acc):
            n = j * ncol + c
            for s in range(2):
                sem = sem_of(n + nw + 2 * nkv, s)
                wait(wo_unit(wo_buf, n, s), sem)
                pl.when(n + _LOOK < nw)(lambda: start_wo(n + _LOOK, s, sem))
            wt = wo_buf[:, :, _ds(j, _BAND), _ds(c, _WC)].reshape(2 * _G * _BAND, _WC)
            return acc + lax.dot_general(lhs_buf[c].astype(bf16), wt, _NT,
                                         preferred_element_type=f32)

        acc = lax.fori_loop(0, ncol, step, zeros)
        acc = jnp.where(lane < _G * _BAND, acc, pltpu.roll(acc, nb, 0))
        acc = pltpu.roll(acc, _divmod(j * _BAND, _DH)[1], 1)
        return [jnp.where(b == j, acc, y) for b, y in zip(band_of_col, ys)]

    ys = lax.fori_loop(0, nband, band, [zeros] * ntile)
    y_buf[...] = jnp.concatenate(ys, axis=1)[0:nb].astype(y_buf.dtype)


def _kernel(*refs):
    ins, out_hbm, bufs, out_sem = refs[:10], refs[10], refs[11:-1], refs[-1]
    out_copy = pltpu.make_async_copy(bufs[-1], out_hbm, out_sem)

    def scoped(x_sem, sems):
        _stream(*ins, *bufs, x_sem, sems)
        out_copy.start()

    pl.run_scoped(scoped, pltpu.SemaphoreType.DMA((2,)), pltpu.SemaphoreType.DMA((2 * _LOOK,)))
    out_copy.wait()


@jax.jit
def pallas_concat_heads__sliding_block_cached__sliding_block_cached__decode_kernel(
    A_x: jax.Array,
    A_k_cache: jax.Array,
    A_v_cache: jax.Array,
    A_wq: jax.Array,
    A_wo: jax.Array,
    B_x: jax.Array,
    B_k_cache: jax.Array,
    B_v_cache: jax.Array,
    B_wq: jax.Array,
    B_wo: jax.Array,
):
    nb, sq, d = A_x.shape
    _, hkv, sk, dh = A_k_cache.shape
    w = min(4096, max(256, sk // 4))
    assert (nb, sq, dh, 2 * hkv) == (_G, 1, _DH, _HQ)
    assert d == _G * (_DH + _BAND) and w == _LOOK * _BLK and sk % _KR == 0
    assert B_x.shape == A_x.shape and B_k_cache.shape == A_k_cache.shape

    f32, bf16 = jnp.float32, jnp.bfloat16
    hbm = pl.BlockSpec(memory_space=pltpu.HBM)

    def heads(a):
        return a.reshape(nb * hkv, sk, dh)

    def quarters(a):
        return a.reshape(_G, d // _G, _HQ * _DH)

    out = pl.pallas_call(
        _kernel,
        out_shape=jax.ShapeDtypeStruct((nb, 2 * d), bf16),
        in_specs=[hbm] * 10,
        out_specs=hbm,
        scratch_shapes=[
            pltpu.VMEM((2, nb, d), bf16),
            pltpu.VMEM((2 * nb, d), f32),
            pltpu.VMEM((2, _G, d // _G, _HQ * _DH), bf16),
            pltpu.VMEM((2, _G, d // _G, _HQ * _DH), bf16),
            pltpu.VMEM((_NSLOT, 2, _G, w, _DH), bf16),
            pltpu.VMEM((2 * nb * _HQ, _DH), f32),
            pltpu.VMEM((w // _BLK, 2 * nb, _DH), f32),
            pltpu.VMEM((2 * nb * _HQ, _DH), f32),
            pltpu.VMEM((_HQ * _DH // _WC, 2 * nb, _WC), f32),
            pltpu.VMEM((4, 2 * nb, _DH), f32),
            pltpu.VMEM((nb, 2 * d), bf16),
            pltpu.SemaphoreType.DMA(()),
        ],
        compiler_params=pltpu.CompilerParams(vmem_limit_bytes=64 * 1024 * 1024),
    )(A_x.reshape(nb, d), heads(A_k_cache), heads(A_v_cache), quarters(A_wq), quarters(A_wo.T),
      B_x.reshape(nb, d), heads(B_k_cache), heads(B_v_cache), quarters(B_wq), quarters(B_wo.T))
    return out.reshape(nb, sq, 2 * d)
```

```python
import functools

import jax
import jax.numpy as jnp
from jax import lax
import jax.experimental.pallas as pl
import jax.experimental.pallas.tpu as pltpu

_HQ = 32
_DH = 128
_G = 4
_BLK = 128
_KR = 64
_WR = 8
_WC = 1024
_BAND = 16
_QC = 256
_LOOK = 16
_NSLOT = 4
_NT = (((1,), (1,)), ((), ()))
_PIECES = ((0, 0, _G - 1, 1), (1, 1, _G - 1, 1), (0, _G - 1, 1, 0), (1, 0, 1, 0))


def _divmod(j, n):
    assert n & (n - 1) == 0
    return lax.shift_right_logical(j, n.bit_length() - 1), j & (n - 1)


def _ds(i, n):
    return pl.ds(i * n if isinstance(i, int) else pl.multiple_of(i * n, n), n)


def _stream(xa, ka, va, wqa, woa, xb, kb, vb, wqb, wob,
            x_buf, x8_buf, wq_buf, wo_buf, kv_buf, q_buf, s_buf, o_buf, lhs_buf,
            st_buf, y_buf, x_sem, sems):
    f32, bf16 = jnp.float32, jnp.bfloat16
    nb, d = xa.shape
    sk, w = ka.shape[1], kv_buf.shape[3]
    rows = 2 * nb
    ngrp = ka.shape[0] // _G
    nblk = w // _BLK
    nkv = ngrp * nblk
    ncol = _HQ * _DH // _WC
    nband = d // _G // _BAND
    nw = nband * ncol

    def w_unit(ref, r, c):
        return ref.at[(slice(None),) * (len(ref.shape) - 2) + (_ds(r, _WR), _ds(c, _WC))]

    def wq_unit(ref, n, s):
        return w_unit(ref, *_divmod(2 * n + s, ncol))

    def wo_unit(ref, n, s):
        r, c = _divmod(n, ncol)
        return w_unit(ref, 2 * r + s, c)

    def kv_dst(n, s):
        g, i = _divmod(n, nblk)
        return kv_buf.at[_divmod(g, _NSLOT)[1], :, :, _ds(2 * i + s, _KR), :]

    def kv_src(ref, n, s):
        g, i = _divmod(n, nblk)
        return ref.at[_ds(g, _G), _ds((sk - w) // _KR + 2 * i + s, _KR), :]

    def start(srcs, dst, sem):
        for a, l0, nl, queue in _PIECES:
            pltpu.make_async_copy(srcs[a].at[pl.ds(l0, nl)], dst.at[a, pl.ds(l0, nl)],
                                  sem).start(priority=queue)

    def wait(dst, sem):
        pltpu.make_async_copy(dst, dst, sem).wait()

    def sem_of(n, s):
        return sems.at[2 * _divmod(n, _LOOK)[1] + s]

    def start_wq(n, s, sem):
        start((wq_unit(wqa, n, s), wq_unit(wqb, n, s)), wq_unit(wq_buf, n, s), sem)

    def start_a(n, s, sem):
        start((kv_src(ka, n, s), kv_src(va, n, s)), kv_dst(n, s), sem)

    def start_b(n, s, sem):
        start((kv_src(kb, n - nkv, s), kv_src(vb, n - nkv, s)), kv_dst(n, s), sem)

    def start_wo(n, s, sem):
        start((wo_unit(woa, n, s), wo_unit(wob, n, s)), wo_unit(wo_buf, n, s), sem)

    x_copies = [pltpu.make_async_copy(x, x_buf.at[i], x_sem.at[i])
                for i, x in enumerate((xa, xb))]

    @pl.loop(0, _LOOK)
    def _(n):
        for s in range(2):
            start_wq(n, s, sem_of(n, s))

    for cp in x_copies:
        cp.start()

    @pl.loop(0, nw - _LOOK)
    def _(n):
        for s in range(2):
            wait(wq_unit(wq_buf, n, s), sem_of(n, s))
            start_wq(n + _LOOK, s, sem_of(n, s))

    @pl.loop(nw - _LOOK, nw)
    def _(n):
        for s in range(2):
            wait(wq_unit(wq_buf, n, s), sem_of(n, s))
            start_a(n - (nw - _LOOK), s, sem_of(n, s))

    for cp in x_copies:
        cp.wait()
    x8_buf[...] = jnp.concatenate([x_buf[0].astype(f32), x_buf[1].astype(f32)], axis=0)

    def q_step(n):
        x8 = x8_buf[...].astype(bf16)
        qa, qb = [jnp.dot(x8, wq_buf[br, :, :, _ds(n, _QC)].reshape(d, _QC),
                          preferred_element_type=f32) for br in range(2)]
        q = jnp.where(lax.broadcasted_iota(jnp.int32, qa.shape, 0) < nb, qa, qb)
        for h in range(_QC // _DH):
            q_buf[pl.ds(n * (_QC // _DH) + h, rows, stride=_HQ), :] = q[:, h * _DH:(h + 1) * _DH]

    nq = _HQ * _DH // _QC
    nq0 = rows * _DH // _QC
    assert nq - nq0 <= nblk
    pl.loop(0, nq0)(q_step)

    zeros = jnp.zeros((rows, _DH), f32)
    neg_inf = jnp.full((rows, _DH), -jnp.inf, f32)
    lane_of_row = lax.shift_right_logical(lax.broadcasted_iota(jnp.int32, (rows, _DH), 0), 1)
    M_PREV, M_RUN, L_ACC, O_ACC = range(4)
    st_buf[M_RUN] = neg_inf

    def pick(parts):
        out = parts[0]
        for l in range(1, _G):
            out = jnp.where(lane_of_row == l, parts[l], out)
        return out

    def pv_step(slot, i):
        e = jnp.exp(s_buf[i] - st_buf[M_PREV])
        p = e.astype(bf16)
        st_buf[L_ACC] += e
        st_buf[O_ACC] += pick([jnp.dot(p, kv_buf[slot, 1, l, _ds(i, _BLK), :],
                                       preferred_element_type=f32) for l in range(_G)])

    def finish(t):
        o_buf[_ds(t, rows), :] = st_buf[O_ACC] / jnp.sum(st_buf[L_ACC], axis=-1, keepdims=True)

    def attend(start_next, first, n):
        t, i = _divmod(n, nblk)

        def advance(s):
            sem = sem_of(n + nw, s)
            wait(kv_dst(n, s), sem)
            start_next(n + _LOOK, s, sem)

        advance(0)
        if first:
            pl.when(i + nq0 < nq)(lambda: q_step(i + nq0))
        else:
            pv_step(_divmod(t - 1, _NSLOT)[1], i)
        advance(1)
        q = q_buf[_ds(t, rows), :].astype(bf16)
        s = pick([lax.dot_general(q, kv_buf[_divmod(t, _NSLOT)[1], 0, l, _ds(i, _BLK), :], _NT,
                                  preferred_element_type=f32)
                  for l in range(_G)]) * (_DH ** -0.5)
        s_buf[i] = s
        st_buf[M_RUN] = jnp.maximum(st_buf[M_RUN], s)

        @pl.when(i == nblk - 1)
        def _():
            if not first:
                finish(t - 1)
            st_buf[M_PREV] = jnp.broadcast_to(
                jnp.max(st_buf[M_RUN], axis=-1, keepdims=True), (rows, _DH))
            st_buf[M_RUN] = neg_inf
            st_buf[L_ACC] = zeros
            st_buf[O_ACC] = zeros

    lo = 0
    for hi, start_next in ((nblk, start_a),
                           (nkv - _LOOK, start_a),
                           (2 * nkv - _LOOK, start_b),
                           (2 * nkv, lambda n, s, sem: start_wo(n - 2 * nkv, s, sem))):
        pl.loop(lo, hi)(functools.partial(attend, start_next, lo == 0))
        lo = hi

    last = 2 * ngrp - 1
    pl.loop(0, nblk, unroll=2)(functools.partial(pv_step, last % _NSLOT))
    finish(last)

    hpc = _WC // _DH
    for c in range(ncol):
        lhs_buf[c] = jnp.concatenate(
            [o_buf[pl.ds(c * hpc + h, rows, stride=_HQ), :] for h in range(hpc)], axis=1)

    ntile = 2 * d // _DH
    lane = lax.broadcasted_iota(jnp.int32, (rows, _DH), 1)
    seg = _divmod(lane, _BAND)[0]
    segs = [seg + (v * _DH // _BAND) % nband for v in range(ntile)]
    band_of_col = [jnp.where(x >= nband, x - nband, x) for x in segs]

    def band(is_last, j, ys):
        def step(c, acc):
            n = j * ncol + c
            for s in range(2):
                sem = sem_of(n + nw + 2 * nkv, s)
                wait(wo_unit(wo_buf, n, s), sem)
                if not is_last:
                    pl.when(n + _LOOK < nw)(lambda: start_wo(n + _LOOK, s, sem))
            wt = wo_buf[:, :, _ds(j, _BAND), _ds(c, _WC)].reshape(2 * _G * _BAND, _WC)
            return acc + lax.dot_general(lhs_buf[c].astype(bf16), wt, _NT,
                                         preferred_element_type=f32)

        acc = lax.fori_loop(0, ncol, step, zeros)
        acc = jnp.where(lane < _G * _BAND, acc, pltpu.roll(acc, nb, 0))
        if not is_last:
            acc = pltpu.roll(acc, j * _BAND, 1)
        return [jnp.where(b == j, acc, y) for b, y in zip(band_of_col, ys)]

    assert (nband - 1) * _BAND == _DH and ncol <= _LOOK
    ys = lax.fori_loop(0, nband - 1, functools.partial(band, False), [zeros] * ntile)
    ys = band(True, nband - 1, ys)
    y_buf[...] = jnp.concatenate(ys, axis=1)[0:nb].astype(y_buf.dtype)


def _kernel(*refs):
    ins, out_hbm, bufs, out_sem = refs[:10], refs[10], refs[11:-1], refs[-1]
    out_copy = pltpu.make_async_copy(bufs[-1], out_hbm, out_sem)

    def scoped(x_sem, sems):
        _stream(*ins, *bufs, x_sem, sems)
        out_copy.start()

    pl.run_scoped(scoped, pltpu.SemaphoreType.DMA((2,)), pltpu.SemaphoreType.DMA((2 * _LOOK,)))
    out_copy.wait()


@jax.jit
def pallas_concat_heads__sliding_block_cached__sliding_block_cached__decode_kernel(
    A_x: jax.Array,
    A_k_cache: jax.Array,
    A_v_cache: jax.Array,
    A_wq: jax.Array,
    A_wo: jax.Array,
    B_x: jax.Array,
    B_k_cache: jax.Array,
    B_v_cache: jax.Array,
    B_wq: jax.Array,
    B_wo: jax.Array,
):
    nb, sq, d = A_x.shape
    _, hkv, sk, dh = A_k_cache.shape
    w = min(4096, max(256, sk // 4))
    assert (nb, sq, dh, 2 * hkv) == (_G, 1, _DH, _HQ)
    assert d == _G * (_DH + _BAND) and w == _LOOK * _BLK and sk % _KR == 0
    assert B_x.shape == A_x.shape and B_k_cache.shape == A_k_cache.shape

    f32, bf16 = jnp.float32, jnp.bfloat16
    hbm = pl.BlockSpec(memory_space=pltpu.HBM)

    def heads(a):
        return a.reshape(nb * hkv, sk, dh)

    def quarters(a):
        return a.reshape(_G, d // _G, _HQ * _DH)

    out = pl.pallas_call(
        _kernel,
        out_shape=jax.ShapeDtypeStruct((nb, 2 * d), bf16),
        in_specs=[hbm] * 10,
        out_specs=hbm,
        scratch_shapes=[
            pltpu.VMEM((2, nb, d), bf16),
            pltpu.VMEM((2 * nb, d), f32),
            pltpu.VMEM((2, _G, d // _G, _HQ * _DH), bf16),
            pltpu.VMEM((2, _G, d // _G, _HQ * _DH), bf16),
            pltpu.VMEM((_NSLOT, 2, _G, w, _DH), bf16),
            pltpu.VMEM((2 * nb * _HQ, _DH), f32),
            pltpu.VMEM((w // _BLK, 2 * nb, _DH), f32),
            pltpu.VMEM((2 * nb * _HQ, _DH), f32),
            pltpu.VMEM((_HQ * _DH // _WC, 2 * nb, _WC), f32),
            pltpu.VMEM((4, 2 * nb, _DH), f32),
            pltpu.VMEM((nb, 2 * d), bf16),
            pltpu.SemaphoreType.DMA(()),
        ],
        compiler_params=pltpu.CompilerParams(vmem_limit_bytes=64 * 1024 * 1024),
    )(A_x.reshape(nb, d), heads(A_k_cache), heads(A_v_cache), quarters(A_wq), quarters(A_wo.T),
      B_x.reshape(nb, d), heads(B_k_cache), heads(B_v_cache), quarters(B_wq), quarters(B_wo.T))
    return out.reshape(nb, sq, 2 * d)
```
